```python
import os as _os
_os.environ.setdefault("JAX_PLATFORMS", "cpu")
import jax
import jax.numpy as jnp

def _softmax(x, axis=-1):
    return jax.nn.softmax(x, axis=axis)
def _gelu(x):
    return jax.nn.gelu(x, approximate=True)
def _silu(x):
    return jax.nn.silu(x)
def _sigmoid(x):
    return jax.nn.sigmoid(x)
def _layernorm(x, axis=-1, eps=1e-5):
    m = jnp.mean(x, axis=axis, keepdims=True)
    v = jnp.var(x, axis=axis, keepdims=True)
    return (x - m) / jnp.sqrt(v + eps)
def _scatter_add(tgt, idx, src, axis=0):
    return tgt.at[idx].add(src)
def _segment_sum(src, seg, n):
    return jax.ops.segment_sum(src, seg, n)
class _Rng:
    def __init__(self, key):
        self._k = key
    def _next(self):
        self._k, sub = jax.random.split(self._k)
        return sub
    def normal(self, shape):
        return jax.random.normal(self._next(), shape, dtype=jnp.bfloat16)
    def randint(self, lo, hi, shape):
        return jax.random.randint(self._next(), shape, lo, hi, dtype=jnp.int32)
    def uniform(self, shape, lo=0.0, hi=1.0):
        return jax.random.uniform(self._next(), shape, jnp.bfloat16, lo, hi)
    def permutation(self, n):
        return jax.random.permutation(self._next(), n)


kernel_name = 'concat_heads__gqa_block_cached__mha_block_cached__near_ridge'

def setup_inputs():
    _rng = _Rng(jax.random.key(int.from_bytes(__import__("os").urandom(4), "little")))
    _w = (lambda a: (lambda t: t.astype(jnp.bfloat16) if jnp.issubdtype(t.dtype, jnp.floating) else t)(jnp.asarray(a)))
    def _A_setup():
        B, Sq, D = 16, 32, 512
        Hq, Hkv, Sk, Dh = 32, 8, 512, 128
        assert Hq % Hkv == 0, (Hq, Hkv)
        return {
            "x": _w((lambda *s: _rng.normal(s) * 0.8)(B, Sq, D)),
            "k_cache": _w((lambda *s: _rng.normal(s) * 0.8)(B, Hkv, Sk, Dh)),
            "v_cache": _w((lambda *s: _rng.normal(s) * 0.05)(B, Hkv, Sk, Dh)),
            "wq": _w((lambda *s: _rng.normal(s) * 0.8)(D, Hq * Dh) * (D ** -0.5)),
            "wo": _w((lambda *s: _rng.normal(s) * 0.05)(Hq * Dh, D) * ((Hq * Dh) ** -0.5)),
        }
    _A_in = _A_setup()

    def _B_setup():
        B, Sq, D = 16, 32, 512
        H, Sk, Dh = 32, 512, 128
        return {
            "x": _w((lambda *s: _rng.normal(s) * 0.8)(B, Sq, D)),
            "k_cache": _w((lambda *s: _rng.normal(s) * 0.8)(B, H, Sk, Dh)),
            "v_cache": _w((lambda *s: _rng.normal(s) * 0.05)(B, H, Sk, Dh)),
            "wq": _w((lambda *s: _rng.normal(s) * 0.8)(D, H * Dh) * (D ** -0.5)),
            "wo": _w((lambda *s: _rng.normal(s) * 0.05)(H * Dh, D) * ((H * Dh) ** -0.5)),
        }
    _B_in = _B_setup()

    return {
        "A_x": _A_in["x"],
        "A_k_cache": _A_in["k_cache"],
        "A_v_cache": _A_in["v_cache"],
        "A_wq": _A_in["wq"],
        "A_wo": _A_in["wo"],
        "B_x": _B_in["x"],
        "B_k_cache": _B_in["k_cache"],
        "B_v_cache": _B_in["v_cache"],
        "B_wq": _B_in["wq"],
        "B_wo": _B_in["wo"],
    }

def reference(A_x, A_k_cache, A_v_cache, A_wq, A_wo, B_x, B_k_cache, B_v_cache, B_wq, B_wo):
    def _A_ref(x, k_cache, v_cache, wq, wo):
        B, Sq, D = x.shape
        Hq, Dh = 32, 128
        Hkv = k_cache.shape[1]
        rep = Hq // Hkv
        q = (lambda x, *d: x.transpose(*d))((x @ wq).reshape(B, Sq, Hq, Dh), 0, 2, 1, 3)
        k = jnp.repeat(k_cache, rep, axis=1)
        v = jnp.repeat(v_cache, rep, axis=1)
        scores = jnp.einsum("bhqd,bhkd->bhqk", q, k) * (Dh ** -0.5)
        p = _softmax(scores, axis=-1)
        o = jnp.einsum("bhqk,bhkd->bhqd", p, v)
        return (lambda x, *d: x.transpose(*d))(o, 0, 2, 1, 3).reshape(B, Sq, Hq * Dh) @ wo

    def _B_ref(x, k_cache, v_cache, wq, wo):
        B, Sq, D = x.shape
        H, Dh = 32, 128
        q = (lambda x, *d: x.transpose(*d))((x @ wq).reshape(B, Sq, H, Dh), 0, 2, 1, 3)
        scores = jnp.einsum("bhqd,bhkd->bhqk", q, k_cache) * (Dh ** -0.5)
        p = _softmax(scores, axis=-1)
        o = jnp.einsum("bhqk,bhkd->bhqd", p, v_cache)
        return (lambda x, *d: x.transpose(*d))(o, 0, 2, 1, 3).reshape(B, Sq, H * Dh) @ wo

    a = _A_ref(A_x, A_k_cache, A_v_cache, A_wq, A_wo)
    b = _B_ref(B_x, B_k_cache, B_v_cache, B_wq, B_wo)
    return jnp.concatenate([a, b], axis=-1)
```

```python
import math

import jax
import jax.numpy as jnp
import jax.experimental.pallas as pl
import jax.experimental.pallas.tpu as pltpu

_HEAD_DIM = 128
_NUM_HEADS = 32
_KV_ROWS = 128
_W_ROWS = 32
_LOOKAHEAD = 3
_NUM_SLOTS = _LOOKAHEAD + 1
_NT_DIMS = (((1,), (1,)), ((), ()))


def _softmax_terms(s):
    m = jnp.max(s, axis=-1, keepdims=True)
    p = jnp.exp2(s - m)
    l = jnp.sum(p, axis=-1, keepdims=True)
    return p.astype(jnp.bfloat16), pltpu.reciprocal(l, approx=False)


def _attention_kernel(
    ax, ak, av, awq, awo, bx, bk, bv, bwq, bwo,
    out,
    xbuf, wbuf, kvbuf, obuf, wsem, kvsem, osem,
):
    batch, sq, d_model = ax.shape
    _, num_groups, sk, dh = ak.shape
    group = bk.shape[1] // num_groups
    group_width = group * dh
    num_units = batch * num_groups
    q_scale = dh**-0.5 * math.log2(math.e)

    def start_kv(u):
        b, g, slot = u // num_groups, u % num_groups, u % _NUM_SLOTS
        slabs = [(ak.at[b, g], av.at[b, g])]
        slabs += [(bk.at[b, g * group + j], bv.at[b, g * group + j]) for j in range(group)]
        for j, kv in enumerate(slabs):
            for r in range(0, sk, _KV_ROWS):
                for t in range(2):
                    pltpu.make_async_copy(
                        kv[t].at[pl.ds(r, _KV_ROWS)],
                        kvbuf.at[slot, t, j, pl.ds(r, _KV_ROWS)],
                        kvsem.at[slot],
                    ).start(priority=t)

    def wait_kv(slot):
        pltpu.make_async_copy(kvbuf.at[slot], kvbuf.at[slot], kvsem.at[slot]).wait()

    def start_weights(g):
        col = pl.multiple_of(g * group_width, group_width)
        for t, (wq, wo) in enumerate(((awq, awo), (bwq, bwo))):
            for r in range(0, d_model, _W_ROWS):
                pltpu.make_async_copy(
                    wq.at[pl.ds(r, _W_ROWS), pl.ds(col, group_width)],
                    wbuf.at[g, 2 * t, pl.ds(r, _W_ROWS)],
                    wsem.at[g],
                ).start(priority=0)
                pltpu.make_async_copy(
                    wo.at[pl.ds(col + r, _W_ROWS)],
                    wbuf.at[g, 2 * t + 1, pl.ds(r, _W_ROWS)],
                    wsem.at[g],
                ).start(priority=1)

    def wait_weights(g):
        pltpu.make_async_copy(wbuf.at[g], wbuf.at[g], wsem.at[g]).wait()

    def project(a, w):
        return jnp.dot(a, w, preferred_element_type=jnp.float32)

    def scores(q, k):
        return jax.lax.dot_general(q, k, _NT_DIMS, preferred_element_type=jnp.float32)

    def head(x, j):
        return x[:, j * dh:(j + 1) * dh]

    def compute_unit(b, g, slot):
        qa = (project(xbuf[0, b], wbuf[g, 0]) * q_scale).astype(jnp.bfloat16)
        qb = (project(xbuf[1, b], wbuf[g, 2]) * q_scale).astype(jnp.bfloat16)
        qa = jnp.concatenate([head(qa, j) for j in range(group)], axis=0)
        sa = scores(qa, kvbuf[slot, 0, 0])
        sb = [scores(head(qb, j), kvbuf[slot, 0, 1 + j]) for j in range(group)]
        pa, ra = _softmax_terms(sa)
        pb = [_softmax_terms(s) for s in sb]
        oa = (project(pa, kvbuf[slot, 1, 0]) * ra).astype(jnp.bfloat16)
        ob = [
            (project(p, kvbuf[slot, 1, 1 + j]) * r).astype(jnp.bfloat16)
            for j, (p, r) in enumerate(pb)
        ]
        oa = jnp.concatenate([oa[j * sq:(j + 1) * sq] for j in range(group)], axis=1)
        ob = jnp.concatenate(ob, axis=1)
        return project(oa, wbuf[g, 1]), project(ob, wbuf[g, 3])

    for b in range(batch):
        pltpu.make_async_copy(ax.at[b], xbuf.at[0, b], wsem.at[0]).start(priority=0)
        pltpu.make_async_copy(bx.at[b], xbuf.at[1, b], wsem.at[0]).start(priority=1)
    for u in range(_LOOKAHEAD):
        start_weights(u)
        start_kv(u)
    pltpu.make_async_copy(xbuf, xbuf, wsem.at[0]).wait()

    bulk_out = pltpu.make_async_copy(
        obuf.at[pl.ds(0, batch - 1)], out.at[pl.ds(0, batch - 1)], osem.at[0]
    )
    last_out = pltpu.make_async_copy(obuf.at[batch - 1], out.at[batch - 1], osem.at[1])

    def batch_body(b, _):
        def unit_body(g, acc):
            u = b * num_groups + g
            slot = u % _NUM_SLOTS
            nxt = u + _LOOKAHEAD

            @pl.when(b == 0)
            def _():
                wait_weights(g)

            wait_kv(slot)

            @pl.when(nxt < num_groups)
            def _():
                start_weights(nxt)

            @pl.when(nxt < num_units)
            def _():
                start_kv(nxt)

            @pl.when(u == num_units - 1)
            def _():
                bulk_out.start()

            ya, yb = compute_unit(b, g, slot)
            return acc[0] + ya, acc[1] + yb

        zero = jnp.zeros((sq, d_model), jnp.float32)
        acc_a, acc_b = jax.lax.fori_loop(0, num_groups, unit_body, (zero, zero))
        obuf[b, :, :d_model] = acc_a.astype(obuf.dtype)
        obuf[b, :, d_model:] = acc_b.astype(obuf.dtype)

    jax.lax.fori_loop(0, batch, batch_body, None)
    last_out.start()
    bulk_out.wait()
    last_out.wait()


@jax.jit
def pallas_concat_heads__gqa_block_cached__mha_block_cached__near_ridge_kernel(
    A_x: jax.Array,
    A_k_cache: jax.Array,
    A_v_cache: jax.Array,
    A_wq: jax.Array,
    A_wo: jax.Array,
    B_x: jax.Array,
    B_k_cache: jax.Array,
    B_v_cache: jax.Array,
    B_wq: jax.Array,
    B_wo: jax.Array,
):
    batch, sq, d_model = A_x.shape
    _, num_groups, sk, dh = A_k_cache.shape
    group = _NUM_HEADS // num_groups
    assert dh == _HEAD_DIM and group * dh == d_model
    assert B_k_cache.shape == (batch, _NUM_HEADS, sk, dh)
    dtype = A_x.dtype

    return pl.pallas_call(
        _attention_kernel,
        in_specs=[pl.BlockSpec(memory_space=pl.ANY)] * 10,
        out_specs=pl.BlockSpec(memory_space=pl.ANY),
        out_shape=jax.ShapeDtypeStruct((batch, sq, 2 * d_model), dtype),
        scratch_shapes=[
            pltpu.VMEM((2, batch, sq, d_model), dtype),
            pltpu.VMEM((num_groups, 4, d_model, group * dh), dtype),
            pltpu.VMEM((_NUM_SLOTS, 2, 1 + group, sk, dh), dtype),
            pltpu.VMEM((batch, sq, 2 * d_model), dtype),
            pltpu.SemaphoreType.DMA((num_groups,)),
            pltpu.SemaphoreType.DMA((_NUM_SLOTS,)),
            pltpu.SemaphoreType.DMA((2,)),
        ],
        compiler_params=pltpu.CompilerParams(
            vmem_limit_bytes=64 * 1024 * 1024,
            disable_bounds_checks=True,
        ),
    )(A_x, A_k_cache, A_v_cache, A_wq, A_wo, B_x, B_k_cache, B_v_cache, B_wq, B_wo)
```

```python
import functools
import math

import jax
import jax.numpy as jnp
import jax.experimental.pallas as pl
import jax.experimental.pallas.tpu as pltpu

_NUM_HEADS = 32
_CHUNK = 16 * 1024
_LOOKAHEAD = 3
_NUM_SLOTS = _LOOKAHEAD + 1
_WEIGHT_STREAMS = 4
_SLAB_ORDER = (0, 2, 4, 1, 3)
_NT_DIMS = (((1,), (1,)), ((), ()))


def _dot(a, b):
    return jnp.dot(a, b, preferred_element_type=jnp.float32)


def _dot_nt(a, b):
    return jax.lax.dot_general(a, b, _NT_DIMS, preferred_element_type=jnp.float32)


def _softmax_times_values(s, v):
    p = jnp.exp2(s - jnp.max(s, axis=-1, keepdims=True))
    inv_sum = 1.0 / jnp.sum(p, axis=-1, keepdims=True)
    return (_dot(p.astype(v.dtype), v) * inv_sum).astype(v.dtype)


def _start(copies):
    for copy, queue in copies:
        copy.start(priority=queue)


def _attention_kernel(
    ax, ak, av, awq, awo, bx, bk, bv, bwq, bwo,
    out,
    x_buf, wq_buf, wo_buf, kv_buf, q_buf, acc_buf, out_buf, sems,
):
    batch, sq, d_model = ax.shape
    _, num_groups, sk, dh = ak.shape
    group = bk.shape[1] // num_groups
    width = group * dh
    num_units = batch * num_groups
    q_scale = dh**-0.5 * math.log2(math.e)
    weight_sem = sems.at[_NUM_SLOTS - 1]
    out_sem = sems.at[(num_units - _NUM_SLOTS) % _NUM_SLOTS]

    def x_copies(b):
        return [
            (pltpu.make_async_copy(x.at[b], x_buf.at[t, b], weight_sem), t)
            for t, x in enumerate((ax, bx))
        ]

    wq_rows = 8
    wq_cols = _CHUNK // wq_rows
    wq_chunks_per_row = awq.shape[1] // wq_cols
    wo_rows = _CHUNK // d_model
    weight_steps = awo.shape[0] // wo_rows // _WEIGHT_STREAMS

    def weight_copies(i):
        copies = []
        for stream in range(_WEIGHT_STREAMS):
            k = stream * weight_steps + i
            row = pl.multiple_of(k // wq_chunks_per_row * wq_rows, wq_rows)
            col = pl.multiple_of(k % wq_chunks_per_row * wq_cols, wq_cols)
            tile = (pl.ds(row, wq_rows), pl.ds(col, wq_cols))
            for t, wq in enumerate((awq, bwq)):
                copies.append(
                    (pltpu.make_async_copy(wq.at[tile], wq_buf.at[(t, *tile)], weight_sem), t)
                )
            rows = pl.ds(pl.multiple_of(k * wo_rows, wo_rows), wo_rows)
            for t, wo in enumerate((awo, bwo)):
                copies.append(
                    (pltpu.make_async_copy(wo.at[rows], wo_buf.at[t, rows], weight_sem), t)
                )
        return copies

    def kv_copies(u):
        b, g, slot = u // num_groups, u % num_groups, u % _NUM_SLOTS
        slabs = [(ak.at[b, g], av.at[b, g])]
        for j in range(group):
            h = g + num_groups * j
            slabs.append((bk.at[b, h], bv.at[b, h]))
        kv_rows = _CHUNK // dh
        return [
            (
                pltpu.make_async_copy(
                    slabs[j][t].at[pl.ds(r, kv_rows)],
                    kv_buf.at[slot, t, j, pl.ds(r, kv_rows)],
                    sems.at[slot],
                ),
                t,
            )
            for r in range(0, sk, kv_rows)
            for j in _SLAB_ORDER
            for t in range(2)
        ]

    def wait_kv(u):
        slot = u % _NUM_SLOTS
        pltpu.make_async_copy(kv_buf.at[slot], kv_buf.at[slot], sems.at[slot]).wait()

    def early_out_copies():
        out_rows = _CHUNK // out.shape[-1]
        pieces = [
            (b, pl.ds(r, out_rows))
            for b in range(batch - 1)
            for r in range(0, sq, out_rows)
        ]
        half = len(pieces) // 2
        return [
            (pltpu.make_async_copy(out_buf.at[piece], out.at[piece], out_sem), t)
            for pair in zip(pieces[:half], pieces[half:])
            for t, piece in enumerate(pair)
        ]

    def weight_slices(g):
        a_slice = pl.ds(pl.multiple_of(g * width, width), width)
        b_slices = [
            pl.ds(pl.multiple_of((g + num_groups * j) * dh, dh), dh)
            for j in range(group)
        ]
        return a_slice, b_slices

    def project_queries(u):
        b, g = u // num_groups, u % num_groups
        a_slice, b_slices = weight_slices(g)
        wq_a = wq_buf[0, :, a_slice]
        q_buf[u % 2, 0] = (_dot(x_buf[0, b], wq_a) * q_scale).astype(q_buf.dtype)
        wq_b = jnp.concatenate([wq_buf[1, :, s] for s in b_slices], axis=1)
        q_buf[u % 2, 1] = (_dot(x_buf[1, b], wq_b) * q_scale).astype(q_buf.dtype)

    def accumulate(b, t, y):
        cols = slice(t * d_model, (t + 1) * d_model)
        y = y + acc_buf[b, :, cols]
        acc_buf[b, :, cols] = y
        out_buf[b, :, cols] = y.astype(out_buf.dtype)

    num_hooks = 2 * (1 + group)

    def run_unit(u, hook=lambda i: None, project_next=True):
        b, g, slot = u // num_groups, u % num_groups, u % _NUM_SLOTS
        a_slice, b_slices = weight_slices(g)

        def query(t, j):
            return q_buf[u % 2, t, :, j * dh:(j + 1) * dh]

        q_a = jnp.concatenate([query(0, j) for j in range(group)], axis=0)
        hook(0)
        s_a = _dot_nt(q_a, kv_buf[slot, 0, 0])
        s_b = []
        for j in range(group):
            hook(1 + j)
            s_b.append(_dot_nt(query(1, j), kv_buf[slot, 0, 1 + j]))
        hook(1 + group)
        if project_next:
            project_queries(u + 1)
        o_a = _softmax_times_values(s_a, kv_buf[slot, 1, 0])
        o_a = jnp.concatenate([o_a[j * sq:(j + 1) * sq] for j in range(group)], axis=1)
        o_b = []
        for j in range(group):
            hook(2 + group + j)
            o_b.append(_softmax_times_values(s_b[j], kv_buf[slot, 1, 1 + j]))
        accumulate(b, 0, _dot(o_a, wo_buf[0, a_slice]))
        wo_b = jnp.concatenate([wo_buf[1, s] for s in b_slices], axis=0)
        accumulate(b, 1, _dot(jnp.concatenate(o_b, axis=1), wo_b))

    pl.loop(0, batch)(lambda b: _start(x_copies(b)))
    pl.loop(0, weight_steps)(lambda i: _start(weight_copies(i)))
    pl.loop(0, _LOOKAHEAD)(lambda u: _start(kv_copies(u)))
    acc_buf[...] = jnp.zeros(acc_buf.shape, acc_buf.dtype)

    @pl.loop(0, batch)
    def _(b):
        for copy, _queue in x_copies(b):
            copy.wait()

    @pl.loop(0, weight_steps)
    def _(i):
        for copy, _queue in weight_copies(i):
            copy.wait()

    project_queries(0)

    @pl.loop(0, num_units - _LOOKAHEAD)
    def _(u):
        wait_kv(u)
        refill = kv_copies(u + _LOOKAHEAD)
        n = len(refill) // num_hooks
        run_unit(u, lambda i: _start(refill[i * n:(i + 1) * n]))

    @pl.loop(num_units - _LOOKAHEAD, num_units - 1)
    def _(u):
        def hook(i):
            if i == num_hooks - 2:
                pl.when(u == num_units - 2)(lambda: _start(early_out_copies()))

        wait_kv(u)
        run_unit(u, hook)

    wait_kv(num_units - 1)
    run_unit(num_units - 1, project_next=False)
    pltpu.make_async_copy(out_buf.at[batch - 1], out.at[batch - 1], out_sem).start()
    pltpu.make_async_copy(out_buf, out, out_sem).wait()


@jax.jit
def pallas_concat_heads__gqa_block_cached__mha_block_cached__near_ridge_kernel(
    A_x: jax.Array,
    A_k_cache: jax.Array,
    A_v_cache: jax.Array,
    A_wq: jax.Array,
    A_wo: jax.Array,
    B_x: jax.Array,
    B_k_cache: jax.Array,
    B_v_cache: jax.Array,
    B_wq: jax.Array,
    B_wo: jax.Array,
):
    batch, sq, d_model = A_x.shape
    _, num_groups, sk, dh = A_k_cache.shape
    group = _NUM_HEADS // num_groups
    assert sorted(_SLAB_ORDER) == list(range(1 + group))
    assert B_k_cache.shape == (batch, _NUM_HEADS, sk, dh)
    dtype = A_x.dtype
    vmem = functools.partial(pltpu.VMEM, dtype=dtype)

    return pl.pallas_call(
        _attention_kernel,
        in_specs=[pl.BlockSpec(memory_space=pl.ANY)] * 10,
        out_specs=pl.BlockSpec(memory_space=pl.ANY),
        out_shape=jax.ShapeDtypeStruct((batch, sq, 2 * d_model), dtype),
        scratch_shapes=[
            vmem((2, batch, sq, d_model)),
            vmem((2, d_model, _NUM_HEADS * dh)),
            vmem((2, _NUM_HEADS * dh, d_model)),
            vmem((_NUM_SLOTS, 2, 1 + group, sk, dh)),
            vmem((2, 2, sq, group * dh)),
            pltpu.VMEM((batch, sq, 2 * d_model), jnp.float32),
            vmem((batch, sq, 2 * d_model)),
            pltpu.SemaphoreType.DMA((_NUM_SLOTS,)),
        ],
        compiler_params=pltpu.CompilerParams(vmem_limit_bytes=64 * 1024 * 1024),
    )(A_x, A_k_cache, A_v_cache, A_wq, A_wo, B_x, B_k_cache, B_v_cache, B_wq, B_wo)
```

```python
import functools
import math

import jax
import jax.numpy as jnp
import jax.experimental.pallas as pl
import jax.experimental.pallas.tpu as pltpu

_NUM_HEADS = 32
_CHUNK = 16 * 1024
_LOOKAHEAD = 3
_NUM_SLOTS = _LOOKAHEAD + 1
_WEIGHT_STREAMS = 4
_SLAB_ORDER = (0, 3, 2, 4, 1)
_TAIL_COPIES = 10
_NT_DIMS = (((1,), (1,)), ((), ()))


def _dot(a, b):
    return jnp.dot(a, b, preferred_element_type=jnp.float32)


def _dot_nt(a, b):
    return jax.lax.dot_general(a, b, _NT_DIMS, preferred_element_type=jnp.float32)


def _softmax_times_values(s, v):
    p = jnp.exp2(s - jnp.max(s, axis=-1, keepdims=True))
    inv_sum = 1.0 / jnp.sum(p, axis=-1, keepdims=True)
    return (_dot(p.astype(v.dtype), v) * inv_sum).astype(v.dtype)


def _start(copies):
    for copy, queue in copies:
        copy.start(priority=queue)


def _wait(copies):
    for copy, _ in copies:
        copy.wait()


def _attention_kernel(
    ax, ak, av, awq, awo, bx, bk, bv, bwq, bwo,
    out,
    x_buf, wq_buf, wo_buf, kv_buf, q_buf, acc_buf, out_buf, sems,
):
    batch, sq, d_model = ax.shape
    _, num_groups, sk, dh = ak.shape
    group = bk.shape[1] // num_groups
    width = group * dh
    num_units = batch * num_groups
    q_scale = dh**-0.5 * math.log2(math.e)
    weight_sem = sems.at[_NUM_SLOTS - 1]
    out_sem = sems.at[(num_units - _NUM_SLOTS) % _NUM_SLOTS]
    last_unit = num_units - 1

    def x_copies(b):
        return [
            (pltpu.make_async_copy(x.at[b], x_buf.at[t, b], weight_sem), t)
            for t, x in enumerate((ax, bx))
        ]

    wq_rows = 8
    wq_cols = _CHUNK // wq_rows
    wq_chunks_per_row = awq.shape[1] // wq_cols
    wo_rows = _CHUNK // d_model
    weight_steps = awo.shape[0] // wo_rows // _WEIGHT_STREAMS

    def weight_copies(i):
        copies = []
        for stream in range(_WEIGHT_STREAMS):
            k = stream * weight_steps + i
            row = pl.multiple_of(k // wq_chunks_per_row * wq_rows, wq_rows)
            col = pl.multiple_of(k % wq_chunks_per_row * wq_cols, wq_cols)
            tile = (pl.ds(row, wq_rows), pl.ds(col, wq_cols))
            for t, wq in enumerate((awq, bwq)):
                copies.append(
                    (pltpu.make_async_copy(wq.at[tile], wq_buf.at[(t, *tile)], weight_sem), t)
                )
            rows = pl.ds(pl.multiple_of(k * wo_rows, wo_rows), wo_rows)
            for t, wo in enumerate((awo, bwo)):
                copies.append(
                    (pltpu.make_async_copy(wo.at[rows], wo_buf.at[t, rows], weight_sem), t)
                )
        return copies

    def kv_copies(u, part=None):
        b, g, slot = u // num_groups, u % num_groups, u % _NUM_SLOTS
        tail_slot = jnp.where(u == last_unit, _NUM_SLOTS, slot)
        slabs = [(ak.at[b, g], av.at[b, g])]
        for j in range(group):
            h = g + num_groups * j
            slabs.append((bk.at[b, h], bv.at[b, h]))
        kv_rows = _CHUNK // dh
        steps = [(r, j) for r in range(0, sk, kv_rows) for j in _SLAB_ORDER]
        copies = []
        for i, (r, j) in enumerate(steps):
            for t in range(2):
                in_tail = t == 1 and i >= len(steps) - _TAIL_COPIES
                if part is None or part == ("tail" if in_tail else "head"):
                    copy = pltpu.make_async_copy(
                        slabs[j][t].at[pl.ds(r, kv_rows)],
                        kv_buf.at[slot, t, j, pl.ds(r, kv_rows)],
                        sems.at[tail_slot if in_tail else slot],
                    )
                    copies.append((copy, t))
        return copies

    def wait_kv(u):
        slot = u % _NUM_SLOTS
        pltpu.make_async_copy(kv_buf.at[slot], kv_buf.at[slot], sems.at[slot]).wait()

    def early_out_copies():
        out_rows = _CHUNK // out.shape[-1]
        pieces = [
            (b, pl.ds(r, out_rows))
            for b in range(batch - 1)
            for r in range(0, sq, out_rows)
        ]
        half = len(pieces) // 2
        return [
            (pltpu.make_async_copy(out_buf.at[piece], out.at[piece], out_sem), t)
            for pair in zip(pieces[:half], pieces[half:])
            for t, piece in enumerate(pair)
        ]

    def weight_slices(g):
        a_slice = pl.ds(pl.multiple_of(g * width, width), width)
        b_slices = [
            pl.ds(pl.multiple_of((g + num_groups * j) * dh, dh), dh)
            for j in range(group)
        ]
        return a_slice, b_slices

    def project_queries(u):
        b, g = u // num_groups, u % num_groups
        a_slice, b_slices = weight_slices(g)
        wq_a = wq_buf[0, :, a_slice]
        q_buf[u % _NUM_SLOTS, 0] = (_dot(x_buf[0, b], wq_a) * q_scale).astype(q_buf.dtype)
        wq_b = jnp.concatenate([wq_buf[1, :, s] for s in b_slices], axis=1)
        q_buf[u % _NUM_SLOTS, 1] = (_dot(x_buf[1, b], wq_b) * q_scale).astype(q_buf.dtype)

    def accumulate(b, t, y):
        cols = slice(t * d_model, (t + 1) * d_model)
        y = y + acc_buf[b, :, cols]
        acc_buf[b, :, cols] = y
        out_buf[b, :, cols] = y.astype(out_buf.dtype)

    num_hooks = 2 * (1 + group)

    def run_unit(u, hook=lambda i: None, project_next=True):
        b, g, slot = u // num_groups, u % num_groups, u % _NUM_SLOTS
        a_slice, b_slices = weight_slices(g)

        def query(t, j):
            return q_buf[u % _NUM_SLOTS, t, :, j * dh:(j + 1) * dh]

        q_a = jnp.concatenate([query(0, j) for j in range(group)], axis=0)
        hook(0)
        s_a = _dot_nt(q_a, kv_buf[slot, 0, 0])
        s_b = []
        for j in range(group):
            hook(1 + j)
            s_b.append(_dot_nt(query(1, j), kv_buf[slot, 0, 1 + j]))
        hook(1 + group)
        if project_next:
            project_queries(u + 1)
        o_a = _softmax_times_values(s_a, kv_buf[slot, 1, 0])
        o_a = jnp.concatenate([o_a[j * sq:(j + 1) * sq] for j in range(group)], axis=1)
        o_b = []
        for j in range(group):
            hook(2 + group + j)
            o_b.append(_softmax_times_values(s_b[j], kv_buf[slot, 1, 1 + j]))
        accumulate(b, 0, _dot(o_a, wo_buf[0, a_slice]))
        wo_b = jnp.concatenate([wo_buf[1, s] for s in b_slices], axis=0)
        accumulate(b, 1, _dot(jnp.concatenate(o_b, axis=1), wo_b))

    pl.loop(0, batch)(lambda b: _start(x_copies(b)))
    pl.loop(0, weight_steps)(lambda i: _start(weight_copies(i)))
    pl.loop(0, _LOOKAHEAD)(lambda u: _start(kv_copies(u)))
    acc_buf[...] = jnp.zeros(acc_buf.shape, acc_buf.dtype)

    pl.loop(0, batch)(lambda b: _wait(x_copies(b)))
    pl.loop(0, weight_steps)(lambda i: _wait(weight_copies(i)))
    project_queries(0)

    @pl.loop(0, num_units - _LOOKAHEAD)
    def _(u):
        wait_kv(u)
        refill = kv_copies(u + _LOOKAHEAD)
        n = len(refill) // num_hooks
        run_unit(u, lambda i: _start(refill[i * n:(i + 1) * n]))

    pl.loop(num_units - _LOOKAHEAD + 1, num_units)(project_queries)

    @pl.loop(num_units - _LOOKAHEAD, num_units)
    def _(u):
        def hook(i):
            if i == num_hooks - 2:
                pl.when(u == last_unit - 1)(lambda: _wait(kv_copies(last_unit, "head")))
                pl.when(u == last_unit - 1)(lambda: _start(early_out_copies()))

        pl.when(u < last_unit)(lambda: wait_kv(u))
        pl.when(u == last_unit)(lambda: _wait(kv_copies(last_unit, "tail")))
        run_unit(u, hook, project_next=False)

    pltpu.make_async_copy(out_buf.at[batch - 1], out.at[batch - 1], out_sem).start()
    pltpu.make_async_copy(out_buf, out, out_sem).wait()


@jax.jit
def pallas_concat_heads__gqa_block_cached__mha_block_cached__near_ridge_kernel(
    A_x: jax.Array,
    A_k_cache: jax.Array,
    A_v_cache: jax.Array,
    A_wq: jax.Array,
    A_wo: jax.Array,
    B_x: jax.Array,
    B_k_cache: jax.Array,
    B_v_cache: jax.Array,
    B_wq: jax.Array,
    B_wo: jax.Array,
):
    batch, sq, d_model = A_x.shape
    _, num_groups, sk, dh = A_k_cache.shape
    group = _NUM_HEADS // num_groups
    assert sorted(_SLAB_ORDER) == list(range(1 + group))
    assert B_k_cache.shape == (batch, _NUM_HEADS, sk, dh)
    dtype = A_x.dtype
    vmem = functools.partial(pltpu.VMEM, dtype=dtype)

    return pl.pallas_call(
        _attention_kernel,
        in_specs=[pl.BlockSpec(memory_space=pl.ANY)] * 10,
        out_specs=pl.BlockSpec(memory_space=pl.ANY),
        out_shape=jax.ShapeDtypeStruct((batch, sq, 2 * d_model), dtype),
        scratch_shapes=[
            vmem((2, batch, sq, d_model)),
            vmem((2, d_model, _NUM_HEADS * dh)),
            vmem((2, _NUM_HEADS * dh, d_model)),
            vmem((_NUM_SLOTS, 2, 1 + group, sk, dh)),
            vmem((_NUM_SLOTS, 2, sq, group * dh)),
            pltpu.VMEM((batch, sq, 2 * d_model), jnp.float32),
            vmem((batch, sq, 2 * d_model)),
            pltpu.SemaphoreType.DMA((_NUM_SLOTS + 1,)),
        ],
        compiler_params=pltpu.CompilerParams(vmem_limit_bytes=64 * 1024 * 1024),
    )(A_x, A_k_cache, A_v_cache, A_wq, A_wo, B_x, B_k_cache, B_v_cache, B_wq, B_wo)
```
